```python
import os as _os
_os.environ.setdefault('JAX_PLATFORMS', 'cpu')
import jax
import jax.numpy as jnp

def _softmax(x, axis=-1):
    return jax.nn.softmax(x, axis=axis)

def _gelu(x):
    return jax.nn.gelu(x, approximate=True)

def _silu(x):
    return jax.nn.silu(x)

def _sigmoid(x):
    return jax.nn.sigmoid(x)

def _layernorm(x, axis=-1, eps=1e-05):
    m = jnp.mean(x, axis=axis, keepdims=True)
    v = jnp.var(x, axis=axis, keepdims=True)
    return (x - m) / jnp.sqrt(v + eps)

def _scatter_add(tgt, idx, src, axis=0):
    return tgt.at[idx].add(src)

def _segment_sum(src, seg, n):
    return jax.ops.segment_sum(src, seg, n)

class _Rng:

    def __init__(self, key):
        self._k = key

    def _next(self):
        self._k, sub = jax.random.split(self._k)
        return sub

    def normal(self, shape):
        return jax.random.normal(self._next(), shape, dtype=jnp.bfloat16)

    def randint(self, lo, hi, shape):
        return jax.random.randint(self._next(), shape, lo, hi, dtype=jnp.int32)

    def uniform(self, shape, lo=0.0, hi=1.0):
        return jax.random.uniform(self._next(), shape, jnp.bfloat16, lo, hi)

    def permutation(self, n):
        return jax.random.permutation(self._next(), n)
kernel_name = 'parallel_sum__memory_aug_recurrent_mem_tr__dense_activation_silu__prompt'

def setup_inputs():
    _rng = _Rng(jax.random.key(int.from_bytes(__import__("os").urandom(4), "little")))
    _w = lambda a: (lambda t: t.astype(jnp.bfloat16) if jnp.issubdtype(t.dtype, jnp.floating) else t)(jnp.asarray(a))

    def _A_setup():
        B, S, Dm = (1, 2048, 448)
        H, Dh = (16, 256)
        M, seg = (8, 32)
        seg = min(seg, S)
        S = S // seg * seg
        return {'x': _w((lambda *s: _rng.normal(s) * 0.05)(B, S, Dm)), 'mem0': _w((lambda *s: _rng.normal(s) * 0.2)(B, M, Dm)), 'Wq': _w((lambda *s: _rng.normal(s) * 0.8)(Dm, H, Dh) * Dm ** (-0.5)), 'Wk': _w((lambda *s: _rng.normal(s) * 0.8)(Dm, H, Dh) * Dm ** (-0.5)), 'Wv': _w((lambda *s: _rng.normal(s) * 0.2)(Dm, H, Dh) * Dm ** (-0.5)), 'Wo': _w((lambda *s: _rng.normal(s) * 0.2)(H, Dh, Dm) * (H * Dh) ** (-0.5)), 'seg_len': seg}
    _A_in = _A_setup()

    def _B_setup():
        B, S, D, F = (1, 2048, 448, 1792)
        return {'x': _w((lambda *s: _rng.normal(s) * 0.05)(B, S, D)), 'w1': _w((lambda *s: _rng.normal(s) * 0.05)(D, F) * D ** (-0.5)), 'w2': _w((lambda *s: _rng.normal(s) * 0.05)(F, D) * F ** (-0.5))}
    _B_in = _B_setup()
    return {'A_x': _A_in['x'], 'A_mem0': _A_in['mem0'], 'A_Wq': _A_in['Wq'], 'A_Wk': _A_in['Wk'], 'A_Wv': _A_in['Wv'], 'A_Wo': _A_in['Wo'], 'A_seg_len': _A_in['seg_len'], 'B_x': _B_in['x'], 'B_w1': _B_in['w1'], 'B_w2': _B_in['w2']}

def reference(A_x, A_mem0, A_Wq, A_Wk, A_Wv, A_Wo, A_seg_len, B_x, B_w1, B_w2):

    def _A_ref(x, mem0, Wq, Wk, Wv, Wo, seg_len):
        B, S, Dm = x.shape
        H, Dh = (Wq.shape[1], Wq.shape[2])
        M = mem0.shape[1]
        scale = Dh ** (-0.5)
        n_seg = S // seg_len
        L = M + seg_len
        idx = jnp.arange(L)
        mask = (idx[:, None] < M) | (idx[:, None] >= idx[None, :])
        mem = mem0
        outs = []
        for s in range(n_seg):
            xs = x[:, s * seg_len:(s + 1) * seg_len, :].copy()
            h = jnp.concatenate([mem, xs], axis=1)
            q = jnp.einsum('btd,dhe->bhte', h, Wq)
            k = jnp.einsum('btd,dhe->bhte', h, Wk)
            v = jnp.einsum('btd,dhe->bhte', h, Wv)
            scores = jnp.einsum('bhqe,bhke->bhqk', q, k) * scale
            scores = jnp.where(mask[None, None], scores, -1000000000.0)
            p = _softmax(scores, axis=-1)
            o = jnp.einsum('bhqk,bhke->bhqe', p, v)
            o = jnp.einsum('bhte,hed->btd', o, Wo)
            mem = o[:, :M, :].copy()
            outs.append(o[:, M:, :])
        return jnp.concatenate(outs, axis=1)

    def _B_ref(x, w1, w2):
        h = jnp.einsum('bsd,df->bsf', x, w1)
        h = _silu(h)
        out = jnp.einsum('bsf,fd->bsd', h, w2)
        return out
    x = A_x
    xn = _layernorm(x, axis=-1)
    return x + _A_ref(xn, A_mem0, A_Wq, A_Wk, A_Wv, A_Wo, A_seg_len) + _B_ref(xn, B_w1, B_w2)
```

```python
import functools

import jax
import jax.numpy as jnp
import jax.experimental.pallas as pl
import jax.experimental.pallas.tpu as pltpu

CHAIN_ROWS = 32


def _kernel(x_ref, mem0_ref, wq_ref, wk_ref, wv_ref, wo_ref, w1_ref, w2_ref, out_ref,
            mem_scr, xn_scr, base_scr, hc_scr, qkvc_scr, qkve_scr, o_scr, oe_scr, wqkv32, wo32,
            *, M, seg_len, G, Rc, H, Dh, eps, scale):
    Re = seg_len - Rc
    L = M + seg_len
    HD = H * Dh
    f32, bf16 = jnp.float32, jnp.bfloat16

    wqkv_p = wqkv32.bitcast(bf16)
    wo_p = wo32.bitcast(bf16)

    @pl.when(pl.program_id(0) == 0)
    def _():
        mem_scr[...] = mem0_ref[...].astype(f32)
        wqkv_p[:, 0:HD] = wq_ref[...]
        wqkv_p[:, HD:2 * HD] = wk_ref[...]
        wqkv_p[:, 2 * HD:3 * HD] = wv_ref[...]
        wo_p[...] = wo_ref[...]

    x = x_ref[...].astype(f32)
    mu = jnp.mean(x, axis=-1, keepdims=True)
    xc = x - mu
    var = jnp.mean(xc * xc, axis=-1, keepdims=True)
    xn = xc * jax.lax.rsqrt(var + eps)
    xn_scr[...] = xn

    h1 = jnp.dot(xn.astype(bf16), w1_ref[...], preferred_element_type=f32)
    h1 = h1 * jax.nn.sigmoid(h1)
    ffn = jnp.dot(h1.astype(bf16), w2_ref[...], preferred_element_type=f32)
    base_scr[...] = x + ffn

    if Re:
        xe = jnp.concatenate(
            [xn[g * seg_len + Rc:(g + 1) * seg_len] for g in range(G)], axis=0)
        qkve_scr[...] = jnp.dot(xe.astype(bf16), wqkv_p[...],
                                preferred_element_type=f32)

    SLOT = 64
    key = jax.lax.broadcasted_iota(jnp.int32, (L, 128), 0)
    lane = jax.lax.broadcasted_iota(jnp.int32, (L, 128), 1)
    qry = jnp.where(lane >= SLOT, lane - SLOT, lane)
    mask_t = jnp.concatenate([(qry < M) | (qry >= key)] * (H // 2), axis=1)
    zeros_dh = jnp.zeros((L, Dh), f32)
    zpad = jnp.zeros((SLOT - L, 2 * Dh), f32)

    def seg_body(g, carry):
        r0 = pl.multiple_of(g * seg_len, seg_len)
        hc_scr[0:M, :] = mem_scr[...]
        hc_scr[M:M + Rc, :] = xn_scr[pl.ds(r0, Rc), :]
        qkvc_scr[...] = jnp.dot(hc_scr[...].astype(bf16), wqkv_p[...],
                                preferred_element_type=f32)
        e0 = pl.multiple_of(g * Re, Re) if Re else 0

        def rows_f32(c0, width):
            blk = qkvc_scr[:, c0:c0 + width]
            if Re:
                blk = jnp.concatenate(
                    [blk, qkve_scr[pl.ds(e0, Re), c0:c0 + width]], axis=0)
            return blk

        sts = []
        for i in range(H // 2):
            h0, h1 = 2 * i, 2 * i + 1
            k2 = rows_f32(HD + h0 * Dh, 2 * Dh).astype(bf16)
            q2bd = jnp.concatenate(
                [jnp.concatenate([rows_f32(h0 * Dh, Dh), zeros_dh], axis=1), zpad,
                 jnp.concatenate([zeros_dh, rows_f32(h1 * Dh, Dh)], axis=1), zpad],
                axis=0).astype(bf16)
            sts.append(jax.lax.dot_general(k2, q2bd, (((1,), (1,)), ((), ())),
                                           preferred_element_type=f32))
        sT = jnp.concatenate(sts, axis=1) * scale
        sT = jnp.where(mask_t, sT, -1e9)
        e = jnp.exp(sT - jnp.max(sT, axis=0, keepdims=True))
        p_all = jnp.transpose(e / jnp.sum(e, axis=0, keepdims=True))
        for h in range(H):
            p0 = (h // 2) * 128 + (h % 2) * SLOT
            oh = jnp.dot(p_all[p0:p0 + L].astype(bf16), rows_f32(2 * HD + h * Dh, Dh).astype(bf16),
                         preferred_element_type=f32)
            o_scr[:, h * Dh:(h + 1) * Dh] = oh[0:M + Rc].astype(o_scr.dtype)
            if Re:
                oe_scr[pl.ds(e0, Re), h * Dh:(h + 1) * Dh] = oh[M + Rc:L]

        o = jnp.dot(o_scr[...], wo_p[...], preferred_element_type=f32)
        mem_scr[...] = o[0:M, :]
        base_scr[pl.ds(r0, Rc), :] = base_scr[pl.ds(r0, Rc), :] + o[M:M + Rc, :]
        return carry

    jax.lax.fori_loop(0, G, seg_body, 0)

    if Re:
        oe = jnp.dot(oe_scr[...].astype(bf16), wo_p[...], preferred_element_type=f32)
        for g in range(G):
            rows = slice(g * seg_len + Rc, (g + 1) * seg_len)
            base_scr[rows, :] = base_scr[rows, :] + oe[g * Re:(g + 1) * Re, :]
    out_ref[...] = base_scr[...].astype(out_ref.dtype)


def _run(A_x, A_mem0, A_Wq, A_Wk, A_Wv, A_Wo, B_w1, B_w2, *, seg_len):
    B, S, Dm = A_x.shape
    assert B == 1
    M = A_mem0.shape[1]
    H, Dh = A_Wq.shape[1], A_Wq.shape[2]
    F = B_w1.shape[1]
    n_seg = S // seg_len
    assert n_seg * seg_len == S and seg_len % 16 == 0 and M % 8 == 0
    assert H % 2 == 0 and M + seg_len <= 64
    L = M + seg_len
    HD = H * Dh

    G = 1
    while G * 2 <= n_seg and n_seg % (G * 2) == 0 and G * 2 * seg_len <= 512:
        G *= 2
    R = G * seg_len
    Rc = min(seg_len, max(CHAIN_ROWS - M, 0))
    Re = seg_len - Rc

    x2 = A_x.reshape(S, Dm)
    mem0 = A_mem0.reshape(M, Dm)
    wo = A_Wo.reshape(HD, Dm)

    kernel = functools.partial(_kernel, M=M, seg_len=seg_len, G=G, Rc=Rc, H=H,
                               Dh=Dh, eps=1e-5, scale=float(Dh) ** (-0.5))
    const = lambda i: (0, 0)
    out = pl.pallas_call(
        kernel,
        grid=(S // R,),
        in_specs=[
            pl.BlockSpec((R, Dm), lambda i: (i, 0)),
            pl.BlockSpec((M, Dm), const),
            pl.BlockSpec((Dm, HD), const),
            pl.BlockSpec((Dm, HD), const),
            pl.BlockSpec((Dm, HD), const),
            pl.BlockSpec((HD, Dm), const),
            pl.BlockSpec((Dm, F), const),
            pl.BlockSpec((F, Dm), const),
        ],
        out_specs=pl.BlockSpec((R, Dm), lambda i: (i, 0)),
        out_shape=jax.ShapeDtypeStruct((S, Dm), A_x.dtype),
        scratch_shapes=[
            pltpu.VMEM((M, Dm), jnp.float32),
            pltpu.VMEM((R, Dm), jnp.float32),
            pltpu.VMEM((R, Dm), jnp.float32),
            pltpu.VMEM((M + Rc, Dm), jnp.float32),
            pltpu.VMEM((M + Rc, 3 * HD), jnp.float32),
            pltpu.VMEM((max(G * Re, 8), 3 * HD), jnp.float32),
            pltpu.VMEM((M + Rc, HD), jnp.bfloat16),
            pltpu.VMEM((max(G * Re, 8), HD), jnp.float32),
            pltpu.VMEM((Dm // 2, 3 * HD), jnp.uint32),
            pltpu.VMEM((HD // 2, Dm), jnp.uint32),
        ],
        compiler_params=pltpu.CompilerParams(
            dimension_semantics=("arbitrary",),
            vmem_limit_bytes=100 * 1024 * 1024,
        ),
    )(x2, mem0, A_Wq.reshape(Dm, HD), A_Wk.reshape(Dm, HD), A_Wv.reshape(Dm, HD), wo, B_w1, B_w2)
    return out.reshape(B, S, Dm)


@functools.partial(jax.jit, static_argnames=("A_seg_len",))
def pallas_parallel_sum__memory_aug_recurrent_mem_tr__dense_activation_silu__prompt_kernel(
    A_x: jax.Array,
    A_mem0: jax.Array,
    A_Wq: jax.Array,
    A_Wk: jax.Array,
    A_Wv: jax.Array,
    A_Wo: jax.Array,
    A_seg_len: int,
    B_x: jax.Array,
    B_w1: jax.Array,
    B_w2: jax.Array,
):
    return _run(A_x, A_mem0, A_Wq, A_Wk, A_Wv, A_Wo, B_w1, B_w2,
                seg_len=int(A_seg_len))
```
